```python
import os as _os
_os.environ.setdefault("JAX_PLATFORMS", "cpu")
import jax
import jax.numpy as jnp

def _softmax(x, axis=-1):
    return jax.nn.softmax(x, axis=axis)
def _gelu(x):
    return jax.nn.gelu(x, approximate=True)
def _silu(x):
    return jax.nn.silu(x)
def _sigmoid(x):
    return jax.nn.sigmoid(x)
def _layernorm(x, axis=-1, eps=1e-5):
    m = jnp.mean(x, axis=axis, keepdims=True)
    v = jnp.var(x, axis=axis, keepdims=True)
    return (x - m) / jnp.sqrt(v + eps)
def _scatter_add(tgt, idx, src, axis=0):
    return tgt.at[idx].add(src)
def _segment_sum(src, seg, n):
    return jax.ops.segment_sum(src, seg, n)
class _Rng:
    def __init__(self, key):
        self._k = key
    def _next(self):
        self._k, sub = jax.random.split(self._k)
        return sub
    def normal(self, shape):
        return jax.random.normal(self._next(), shape, dtype=jnp.bfloat16)
    def randint(self, lo, hi, shape):
        return jax.random.randint(self._next(), shape, lo, hi, dtype=jnp.int32)
    def uniform(self, shape, lo=0.0, hi=1.0):
        return jax.random.uniform(self._next(), shape, jnp.bfloat16, lo, hi)
    def permutation(self, n):
        return jax.random.permutation(self._next(), n)


kernel_name = 'standalone__channel_attn_cbam__vision'

def setup_inputs():
    _rng = _Rng(jax.random.key(int.from_bytes(__import__("os").urandom(4), "little")))
    _w = (lambda a: (lambda t: t.astype(jnp.bfloat16) if jnp.issubdtype(t.dtype, jnp.floating) else t)(jnp.asarray(a)))
    H = W = 224
    C = 192
    r = max(C // 4, 1)
    return {
        "x": _w((lambda *s: _rng.normal(s) * 0.2)(1, H, W, C) + (lambda *s: _rng.normal(s) * 0.2)(1, 1, 1, C) * 2.0),
        "w1": _w((lambda *s: _rng.normal(s) * 0.2)(C, r)),
        "w2": _w((lambda *s: _rng.normal(s) * 0.2)(r, C)),
    }

def reference(x, w1, w2):
    B, H, W, C = x.shape
    xf = x.reshape(B, H * W, C)
    gap = jnp.mean(xf, 1)
    gmp = jnp.amax(xf, 1)
    h_a = gap @ w1
    h_a = h_a * (lambda x, dt: x.astype(dt))(h_a > 0, h_a.dtype)
    h_m = gmp @ w1
    h_m = h_m * (lambda x, dt: x.astype(dt))(h_m > 0, h_m.dtype)
    scale = _sigmoid(h_a @ w2 + h_m @ w2)
    return x * scale[:, None, None, :]
```

```python
import jax
import jax.numpy as jnp
from jax import lax
import jax.experimental.pallas as pl
import jax.experimental.pallas.tpu as pltpu

G = 16
CB = 64


@jax.jit
def pallas_standalone__channel_attn_cbam__vision_kernel(x, w1, w2):
    B, H, W, C = x.shape
    R = w1.shape[1]
    NG = H // G
    rds = [(0, 8, 0, G), (8, 4, 0, G), (12, 1, 0, G), (13, 1, 0, 11), (13, 1, 11, 4), (13, 1, 15, 1)]
    inv_n = 1.0 / (H * W)

    def kernel(x_hbm, w1t_hbm, w2_hbm, o_hbm, buf, w1v, w2v, acc_s, acc_m, scale, sem_in, sem_w, sem_out):
        def rd(i):
            g0, ng, r0, nr = rds[i]
            p = (pl.ds(g0, ng), pl.ds(r0, nr))
            return pltpu.make_async_copy(x_hbm.at[p], buf.at[p], sem_in.at[i])

        cw1 = pltpu.make_async_copy(w1t_hbm, w1v, sem_w.at[0])
        cw2 = pltpu.make_async_copy(w2_hbm, w2v, sem_w.at[1])
        for i in range(len(rds)):
            rd(i).start()

        acc_s[...] = jnp.zeros((C, W), jnp.float32)
        acc_m[...] = jnp.full((C, W), -jnp.inf, jnp.float32)

        for i, (g0, ng, r0, nr) in enumerate(rds):
            rd(i).wait()
            if i == 0:
                cw1.start(priority=1)
                cw2.start(priority=1)

            def cg_body(cg, _):
                cs = pl.ds(pl.multiple_of(cg * 16, 16), 16)

                def rows(g, carry):
                    s, m = carry
                    for r in range(r0, r0 + nr):
                        v = buf[g, r, cs, :].astype(jnp.float32)
                        s = s + v
                        m = jnp.maximum(m, v)
                    return s, m

                init = (acc_s[cs, :], acc_m[cs, :])
                if ng == 1:
                    s, m = rows(g0, init)
                else:
                    s, m = lax.fori_loop(g0, g0 + ng, rows, init)
                acc_s[cs, :] = s
                acc_m[cs, :] = m
                return 0

            lax.fori_loop(0, C // 16, cg_body, 0, unroll=(nr * ng <= 4))
        cw1.wait()
        cw2.wait()

        gap = (jnp.sum(acc_s[...], axis=1, keepdims=True) * inv_n).astype(jnp.bfloat16)
        gmp = jnp.max(acc_m[...], axis=1, keepdims=True).astype(jnp.bfloat16)
        ga = jnp.broadcast_to(gap, (C, 128))
        gm = jnp.broadcast_to(gmp, (C, 128))
        w1t = w1v[...]
        ha = jnp.dot(w1t, ga, preferred_element_type=jnp.float32).astype(jnp.bfloat16).astype(jnp.float32)
        hm = jnp.dot(w1t, gm, preferred_element_type=jnp.float32).astype(jnp.bfloat16).astype(jnp.float32)
        ha = (ha * (ha > 0).astype(jnp.float32)).astype(jnp.bfloat16)
        hm = (hm * (hm > 0).astype(jnp.float32)).astype(jnp.bfloat16)
        w2 = w2v[...]
        dn = (((0,), (0,)), ((), ()))
        sa = lax.dot_general(w2, ha, dn, preferred_element_type=jnp.float32)
        sm = lax.dot_general(w2, hm, dn, preferred_element_type=jnp.float32)
        z = sa + sm
        sc = (1.0 / (1.0 + jnp.exp(-z))).astype(jnp.bfloat16).astype(jnp.float32)
        scale[...] = jnp.concatenate([sc, sc[:, : W - 128]], axis=1)

        def j_body(j, _):
            def cb_body(cb, _):
                def q_body(q, _):
                    cs = pl.ds(pl.multiple_of(cb * CB + q * 16, 16), 16)
                    sv = scale[cs, :]
                    for t in range(NG):
                        buf[t, j, cs, :] = (buf[t, j, cs, :].astype(jnp.float32) * sv).astype(jnp.bfloat16)
                    return 0

                lax.fori_loop(0, CB // 16, q_body, 0)
                p = (slice(None), j, pl.ds(pl.multiple_of(cb * CB, CB), CB))
                pltpu.make_async_copy(buf.at[p], o_hbm.at[p], sem_out.at[0]).start()
                return 0

            lax.fori_loop(0, C // CB, cb_body, 0)
            return 0

        lax.fori_loop(0, G, j_body, 0)
        pltpu.make_async_copy(buf, buf, sem_out.at[0]).wait()

    xt = x.reshape(H, W, C).transpose(0, 2, 1).reshape(NG, G, C, W)
    o = pl.pallas_call(
        kernel,
        out_shape=jax.ShapeDtypeStruct((NG, G, C, W), x.dtype),
        in_specs=[pl.BlockSpec(memory_space=pl.ANY)] * 3,
        out_specs=pl.BlockSpec(memory_space=pl.ANY),
        scratch_shapes=[
            pltpu.VMEM((NG, G, C, W), jnp.bfloat16),
            pltpu.VMEM((R, C), jnp.bfloat16),
            pltpu.VMEM((R, C), jnp.bfloat16),
            pltpu.VMEM((C, W), jnp.float32),
            pltpu.VMEM((C, W), jnp.float32),
            pltpu.VMEM((C, W), jnp.float32),
            pltpu.SemaphoreType.DMA((len(rds),)),
            pltpu.SemaphoreType.DMA((2,)),
            pltpu.SemaphoreType.DMA((1,)),
        ],
        compiler_params=pltpu.CompilerParams(vmem_limit_bytes=64 * 1024 * 1024),
    )(xt, w1.T, w2)
    return o.reshape(H, C, W).transpose(0, 2, 1).reshape(B, H, W, C)
```

```python
import jax
import jax.numpy as jnp
from jax import lax
import jax.experimental.pallas as pl
import jax.experimental.pallas.tpu as pltpu

U = 16
LANES = 128
G = 32
RB = 8

GROUP_READS = (4, 2)
TAIL = 16
TAIL_READS = (7, 3, 1, 1)

WRITE_UNITS = 3
HEAD = 3


def _tree(op, xs):
    while len(xs) > 1:
        xs = [op(*xs[i:i + 2]) if i + 1 < len(xs) else xs[i] for i in range(0, len(xs), 2)]
    return xs[0]


def _round_bf16(v):
    return v.astype(jnp.bfloat16).astype(jnp.float32)


def _cbam_kernel(x_hbm, w1t_hbm, w2_hbm, o_hbm,
                 buf, w1_raw, w2_raw, w1c, w2c, acc_sum, acc_max, scale, sems):
    NG, _, C, W = buf.shape
    R = w1_raw.shape[0]
    NU = C // U
    top = G - TAIL

    pieces = []
    start = 0
    for n in GROUP_READS:
        pieces.append((pl.ds(start, n),))
        start += n
    pieces.append((NG - 1, pl.ds(0, top)))
    start = 0
    for n in TAIL_READS:
        pieces.append((NG - 1, pl.ds(top, TAIL), pl.ds(start * U, n * U)))
        start += n

    slots = [0, 1, 0, 1, 2]
    while len(slots) < len(pieces):
        slots.append(slots[-3])
    reads = [pltpu.make_async_copy(x_hbm.at[p], buf.at[p], sems.at[s])
             for p, s in zip(pieces, slots)]
    weights = [pltpu.make_async_copy(w1t_hbm, w1_raw, sems.at[2]),
               pltpu.make_async_copy(w2_hbm, w2_raw, sems.at[2])]

    def wait_read(i):
        reads[i].wait()
        successor = i + 2 if i < 2 else i + 3
        if successor < len(reads):
            reads[successor].start()

    def pixels(g, r, cs):
        return buf[g, r, cs, :].astype(jnp.float32)

    def pool_rows(carry, cs, g, r0, n):
        s, m = carry
        for r in range(n):
            v = pixels(g, r0 + r, cs)
            s, m = s + v, jnp.maximum(m, v)
        return s, m

    def pool_group(carry, cs, g, n):
        return lax.fori_loop(
            0, n // RB, lambda b, c: pool_rows(c, cs, g, b * RB, RB), carry)

    def channel_rows(w):
        w = w.astype(jnp.float32)
        return jnp.concatenate([w, jnp.zeros((LANES - R, C), jnp.float32)], axis=0).T

    reads[0].start()
    for copy in weights:
        copy.start()
    reads[1].start()

    g0 = 0
    for i in range(len(GROUP_READS) + 1):
        wait_read(i)
        if i == 1:
            for copy in weights:
                copy.wait()
            reads[4].start()
            w1c[...] = channel_rows(w1_raw[...])
            w2c[...] = channel_rows(w2_raw[...])

        def pool_unit(u, _, i=i, g0=g0):
            cs = pl.ds(pl.multiple_of(u * U, U), U)
            if i == 0:
                carry = (jnp.zeros((U, W), jnp.float32),
                         jnp.full((U, W), -jnp.inf, jnp.float32))
            else:
                carry = acc_sum[cs, :], acc_max[cs, :]
            if i < len(GROUP_READS):
                carry = lax.fori_loop(g0, g0 + GROUP_READS[i],
                                      lambda g, c: pool_group(c, cs, g, G), carry)
            else:
                carry = pool_group(carry, cs, NG - 1, top)
            acc_sum[cs, :], acc_max[cs, :] = carry

        lax.fori_loop(0, NU, pool_unit, None)
        if i < len(GROUP_READS):
            g0 += GROUP_READS[i]

    pre_avg = jnp.zeros((8, LANES), jnp.float32)
    pre_max = jnp.zeros((8, LANES), jnp.float32)
    u0 = 0
    for k, n in enumerate(TAIL_READS):
        wait_read(len(GROUP_READS) + 1 + k)
        for u in range(u0, u0 + n):
            cs = pl.ds(u * U, U)
            s, m = acc_sum[cs, :], acc_max[cs, :]
            if u < NU - 1:
                s, m = pool_rows((s, m), cs, NG - 1, top, TAIL)
            else:
                vs = [pixels(NG - 1, top + r, cs) for r in range(TAIL)]
                s, m = _tree(jnp.add, [s] + vs), _tree(jnp.maximum, [m] + vs)
            avg = _round_bf16(jnp.sum(s, axis=1, keepdims=True) * (1.0 / (NG * G * W)))
            mx = jnp.max(m, axis=1, keepdims=True)
            w = w1c[cs, :]
            t_avg, t_max = w * avg, w * mx
            pre_avg = pre_avg + t_avg[:8] + t_avg[8:]
            pre_max = pre_max + t_max[:8] + t_max[8:]
        u0 += n

    h_avg = _round_bf16(jnp.sum(pre_avg, axis=0, keepdims=True))
    h_max = _round_bf16(jnp.sum(pre_max, axis=0, keepdims=True))
    hidden = (h_avg * (h_avg > 0).astype(jnp.float32)
              + h_max * (h_max > 0).astype(jnp.float32))

    def gate(cs):
        z = jnp.sum(w2c[cs, :] * hidden, axis=1, keepdims=True)
        return jnp.broadcast_to(_round_bf16(jax.nn.sigmoid(z)), (cs.size, W))

    def rescale(r, cs, sc):
        for g in range(NG):
            buf[g, r, cs, :] = (pixels(g, r, cs) * sc).astype(buf.dtype)

    def send(r, cs):
        p = (slice(None), r, cs)
        pltpu.make_async_copy(buf.at[p], o_hbm.at[p], sems.at[0]).start()

    first = pl.ds(0, U)
    first_scale = gate(first)

    def send_first_unit(r, _):
        rescale(r, first, first_scale)
        send(r, first)

    send_first_unit(0, None)
    lax.fori_loop(1, HEAD, send_first_unit, None)

    scale[first, :] = first_scale
    rest = pl.ds(U, C - U)
    scale[rest, :] = gate(rest)

    def send_row(r, _, skip=0):
        for lo in range(0, NU, WRITE_UNITS):
            lo, hi = max(lo, skip), lo + WRITE_UNITS
            for u in range(lo, hi):
                cs = pl.ds(u * U, U)
                rescale(r, cs, scale[cs, :])
            send(r, pl.ds(lo * U, (hi - lo) * U))

    lax.fori_loop(0, HEAD, lambda r, c: send_row(r, c, skip=1), None)
    lax.fori_loop(HEAD, G, send_row, None)
    pltpu.make_async_copy(buf, buf, sems.at[0]).wait()


@jax.jit
def pallas_standalone__channel_attn_cbam__vision_kernel(
    x: jax.Array,
    w1: jax.Array,
    w2: jax.Array,
):
    B, H, W, C = x.shape
    R = w1.shape[1]
    NG = H // G
    assert B == 1 and NG * G == H and NG == sum(GROUP_READS) + 1
    assert C == sum(TAIL_READS) * U and (C // U) % WRITE_UNITS == 0 and R <= LANES

    xt = x.reshape(H, W, C).transpose(0, 2, 1).reshape(NG, G, C, W)
    out = pl.pallas_call(
        _cbam_kernel,
        out_shape=jax.ShapeDtypeStruct((NG, G, C, W), x.dtype),
        in_specs=[pl.BlockSpec(memory_space=pl.ANY)] * 3,
        out_specs=pl.BlockSpec(memory_space=pl.ANY),
        scratch_shapes=[
            pltpu.VMEM((NG, G, C, W), x.dtype),
            pltpu.VMEM((R, C), w1.dtype),
            pltpu.VMEM((R, C), w2.dtype),
            pltpu.VMEM((C, LANES), jnp.float32),
            pltpu.VMEM((C, LANES), jnp.float32),
            pltpu.VMEM((C, W), jnp.float32),
            pltpu.VMEM((C, W), jnp.float32),
            pltpu.VMEM((C, W), jnp.float32),
            pltpu.SemaphoreType.DMA((3,)),
        ],
        compiler_params=pltpu.CompilerParams(vmem_limit_bytes=64 * 1024 * 1024),
    )(xt, w1.T, w2)
    return out.reshape(H, C, W).transpose(0, 2, 1).reshape(B, H, W, C)
```
